```python
import jax
import jax.numpy as jnp

def _softmax(x, axis=-1):
    return jax.nn.softmax(x, axis=axis)
def _gelu(x):
    return jax.nn.gelu(x, approximate=True)
def _silu(x):
    return jax.nn.silu(x)
def _sigmoid(x):
    return jax.nn.sigmoid(x)
def _layernorm(x, axis=-1, eps=1e-5):
    m = jnp.mean(x, axis=axis, keepdims=True)
    v = jnp.var(x, axis=axis, keepdims=True)
    return (x - m) / jnp.sqrt(v + eps)
def _scatter_add(tgt, idx, src, axis=0):
    return tgt.at[idx].add(src)
def _segment_sum(src, seg, n):
    return jax.ops.segment_sum(src, seg, n)
class _Rng:
    def __init__(self, key):
        self._k = key
    def _next(self):
        self._k, sub = jax.random.split(self._k)
        return sub
    def normal(self, shape):
        return jax.random.normal(self._next(), shape, dtype=jnp.bfloat16)
    def randint(self, lo, hi, shape):
        return jax.random.randint(self._next(), shape, lo, hi, dtype=jnp.int32)
    def uniform(self, shape, lo=0.0, hi=1.0):
        return jax.random.uniform(self._next(), shape, jnp.bfloat16, lo, hi)
    def permutation(self, n):
        return jax.random.permutation(self._next(), n)


kernel_name = 'gated_mix__sliding_local_dilated__glu_gated_reglu__prompt'

def setup_inputs():
    _rng = _Rng(jax.random.key(int.from_bytes(__import__("os").urandom(4), "little")))
    _w = (lambda a: (lambda t: t.astype(jnp.bfloat16) if jnp.issubdtype(t.dtype, jnp.floating) else t)(jnp.asarray(a)))
    def _A_setup():
        B, S, D = 1, 2048, 1024
        return {
            "x": _w((lambda *s: _rng.normal(s) * 0.05)(B, S, D)),
            "wqkv": _w((lambda *s: _rng.normal(s) * 0.05)(D, 3 * D)),
            "wo": _w((lambda *s: _rng.normal(s) * 0.05)(D, D)),
        }
    _A_in = _A_setup()

    def _B_setup():
        B, S, D, F = 1, 2048, 1024, 3584
        return {
            "x": _w((lambda *s: _rng.normal(s) * 0.05)(B, S, D)),
            "W_gate": _w((lambda *s: _rng.normal(s) * 0.05)(D, F) * (2.0 / D) ** 0.5),
            "W_up": _w((lambda *s: _rng.normal(s) * 0.05)(D, F) * (2.0 / D) ** 0.5),
            "W_down": _w((lambda *s: _rng.normal(s) * 0.05)(F, D) * (1.0 / F) ** 0.5),
        }
    _B_in = _B_setup()

    return {
        "A_x": _A_in["x"],
        "A_wqkv": _A_in["wqkv"],
        "A_wo": _A_in["wo"],
        "B_x": _B_in["x"],
        "B_W_gate": _B_in["W_gate"],
        "B_W_up": _B_in["W_up"],
        "B_W_down": _B_in["W_down"],
        "gate_w": _w((lambda *s: _rng.normal(s) * 0.05)(1024)),
    }

def reference(A_x, A_wqkv, A_wo, B_x, B_W_gate, B_W_up, B_W_down, gate_w):
    def _A_ref(x, wqkv, wo):
        B, S, D = x.shape
        H = 32; Dh = D // H
        W, dil = 8, 2
        qkv = (lambda x, *d: x.transpose(*d))((x @ wqkv).reshape(B, S, 3, H, Dh), 2, 0, 3, 1, 4)
        q, k, v = qkv[0], qkv[1], qkv[2]
        scale = Dh ** -0.5
        pos = jnp.arange(S)
        off = jnp.arange(W) * dil
        idx = pos[:, None] - off[None, :]
        mask = idx >= 0
        idx_c = jnp.where(mask, idx, 0).reshape(-1)
        kg = k[:, :, idx_c, :].reshape(B, H, S, W, Dh)
        vg = v[:, :, idx_c, :].reshape(B, H, S, W, Dh)
        logits = jnp.einsum("bhsd,bhswd->bhsw", q, kg) * scale
        logits = jnp.where(mask[None, None, :, :], logits, -1e9)
        attn = _softmax(logits, axis=-1)
        o = jnp.einsum("bhsw,bhswd->bhsd", attn, vg)
        return (lambda x, *d: x.transpose(*d))(o, 0, 2, 1, 3).reshape(B, S, D) @ wo

    def _B_ref(x, W_gate, W_up, W_down):
        gate = jnp.einsum("bsd,df->bsf", x, W_gate)
        up = jnp.einsum("bsd,df->bsf", x, W_up)
        gate = gate * (lambda x, dt: x.astype(dt))(gate > 0, gate.dtype)
        h = gate * up
        return jnp.einsum("bsf,fd->bsd", h, W_down)

    x = A_x
    g = _sigmoid((x * gate_w).sum(-1, keepdims=True))
    a = _A_ref(x, A_wqkv, A_wo)
    b = _B_ref(x, B_W_gate, B_W_up, B_W_down)
    return g * a + (1 - g) * b
```

```python
import jax
import jax.numpy as jnp
from jax import lax
import jax.experimental.pallas as pl
import jax.experimental.pallas.tpu as pltpu

S = 2048
D = 1024
F = 3584
H = 32
DH = 32
WIN = 8
NCH = D // 128
NA = S // 16
RB = 256
NRB = S // RB
FC = 512
NFC = F // FC
MB = 512
NMB = S // MB
SCALE = DH ** -0.5


def _qkv_chunk(x_v, wqkv_v, dst, c):
    co = pl.multiple_of(c * 128, 128)
    for t in range(3):
        w = wqkv_v[:, pl.ds(t * D + co, 128)]
        for m in range(NMB):
            r = jnp.dot(x_v[pl.ds(m * MB, MB), :], w,
                        preferred_element_type=jnp.float32)
            dst[t, pl.ds(m * MB, MB), :] = r


def _attention_chunk(src, tq, tk, tv, o32, o_v, c):
    lane = lax.broadcasted_iota(jnp.int32, (8, NA), 1)
    first = lane == 0
    for j in range(16):
        rows = pl.ds(j, NA, stride=16)
        tq[j] = (src[0, rows, :] * SCALE).T
        kt = src[1, rows, :].T
        vt = src[2, rows, :].T
        tk[0, j] = kt
        tv[0, j] = vt
        if j >= 2:
            tk[1, j] = pltpu.roll(kt, 1, 1)
            tv[1, j] = pltpu.roll(vt, 1, 1)
    for j in range(16):
        b, p = divmod(j, 2)
        srcs = []
        for w in range(WIN):
            if b >= w:
                srcs.append((0, 2 * (b - w) + p))
            else:
                srcs.append((1, 2 * (b - w + 8) + p))
        outs = []
        for h in range(4):
            hs = pl.ds(h * DH, DH)
            q = tq[j, hs, :]
            lg = []
            for (sh, jj) in srcs:
                pr = q * tk[sh, jj, hs, :]
                pr = (pr[0:8] + pr[8:16]) + (pr[16:24] + pr[24:32])
                l = jnp.broadcast_to(jnp.sum(pr, axis=0, keepdims=True), (8, NA))
                if sh:
                    l = jnp.where(first, jnp.float32(-1e9), l)
                lg.append(l)
            mx = lg[0]
            for l in lg[1:]:
                mx = jnp.maximum(mx, l)
            es = [jnp.exp(l - mx) for l in lg]
            den = es[0]
            for e in es[1:]:
                den = den + e
            inv = 1.0 / den
            acc = [None] * 4
            for (sh, jj), e in zip(srcs, es):
                vv = tv[sh, jj, hs, :]
                for r in range(4):
                    t = e * vv[r * 8:(r + 1) * 8]
                    acc[r] = t if acc[r] is None else acc[r] + t
            outs.extend([a_ * inv for a_ in acc])
        oj = jnp.concatenate(outs, axis=0)
        o32[pl.ds(j, NA, stride=16), :] = oj.T
    co = pl.multiple_of(c * 128, 128)
    o_v[:, pl.ds(co, 128)] = o32[...].astype(jnp.bfloat16)


def _kernel(x_h, wqkv_h, wo_h, wg_h, wu_h, wd_h, gw_ref, out_h,
            x_v, wqkv_v, wo_v, wg_v, wu_v, wd_v, o_v, out_v,
            bufa, bufb, tq, tk, tv, o32, sems, osem):
    def cp(hbm, vm, i):
        return pltpu.make_async_copy(hbm, vm, sems.at[i])

    def wq_cp(t, c):
        cs = pl.ds(t * D + c * 128, 128)
        return [cp(wqkv_h.at[:, cs], wqkv_v.at[:, cs], t)] if c == 0 else []

    c_x = cp(x_h, x_v, 3)
    c_q0 = [cp(wqkv_h.at[:, pl.ds(t * D, 128)], wqkv_v.at[:, pl.ds(t * D, 128)], t)
            for t in range(3)]
    c_qr = [cp(wqkv_h.at[:, pl.ds(t * D + 128, D - 128)],
               wqkv_v.at[:, pl.ds(t * D + 128, D - 128)], 4 + t) for t in range(3)]
    c_wg = cp(wg_h, wg_v, 7)
    c_wu = cp(wu_h, wu_v, 8)
    c_wd = cp(wd_h, wd_v, 9)
    c_wo = cp(wo_h, wo_v, 10)
    for c_ in c_q0:
        c_.start()
    c_x.start()
    for c_ in c_qr:
        c_.start()
    c_wg.start()
    c_wu.start()
    c_wd.start()
    c_wo.start()

    for c_ in c_q0:
        c_.wait()
    c_x.wait()
    _qkv_chunk(x_v, wqkv_v, bufa, 0)
    for c_ in c_qr:
        c_.wait()

    def pair(i, carry):
        c = 2 * i
        _qkv_chunk(x_v, wqkv_v, bufb, c + 1)
        _attention_chunk(bufa, tq, tk, tv, o32, o_v, c)
        _qkv_chunk(x_v, wqkv_v, bufa, c + 2)
        _attention_chunk(bufb, tq, tk, tv, o32, o_v, c + 1)
        return carry

    lax.fori_loop(0, NCH // 2 - 1, pair, 0)
    _qkv_chunk(x_v, wqkv_v, bufb, NCH - 1)
    _attention_chunk(bufa, tq, tk, tv, o32, o_v, NCH - 2)
    _attention_chunk(bufb, tq, tk, tv, o32, o_v, NCH - 1)

    c_wg.wait()
    c_wu.wait()
    c_wd.wait()
    c_wo.wait()

    def out_cp(i):
        rs = pl.ds(pl.multiple_of(i * RB, RB), RB)
        return pltpu.make_async_copy(out_v.at[rs, :], out_h.at[rs, :], osem)

    def ffn(i, carry):
        rs = pl.ds(pl.multiple_of(i * RB, RB), RB)
        xb = x_v[rs, :]
        z = jnp.sum(xb.astype(jnp.float32) * gw_ref[...].astype(jnp.float32),
                    axis=-1, keepdims=True)
        g = jax.nn.sigmoid(z)
        hs = []
        for fc in range(NFC):
            cs = pl.ds(fc * FC, FC)
            gt = jnp.dot(xb, wg_v[:, cs], preferred_element_type=jnp.float32)
            up = jnp.dot(xb, wu_v[:, cs], preferred_element_type=jnp.float32)
            hs.append((jnp.maximum(gt, 0.0) * up).astype(jnp.bfloat16))
        hh = jnp.concatenate(hs, axis=1)
        bb = jnp.dot(hh, wd_v[...], preferred_element_type=jnp.float32)
        aa = jnp.dot(o_v[rs, :], wo_v[...], preferred_element_type=jnp.float32)
        out_v[rs, :] = (g * aa + (1.0 - g) * bb).astype(jnp.bfloat16)
        out_cp(i).start()
        return carry

    lax.fori_loop(0, NRB, ffn, 0)
    pltpu.make_async_copy(out_v, out_h, osem).wait()


@jax.jit
def pallas_gated_mix__sliding_local_dilated__glu_gated_reglu__prompt_kernel(
    A_x: jax.Array,
    A_wqkv: jax.Array,
    A_wo: jax.Array,
    B_x: jax.Array,
    B_W_gate: jax.Array,
    B_W_up: jax.Array,
    B_W_down: jax.Array,
    gate_w: jax.Array,
):
    del B_x
    bf = jnp.bfloat16
    f32 = jnp.float32
    hbm = pl.BlockSpec(memory_space=pl.ANY)
    out = pl.pallas_call(
        _kernel,
        in_specs=[hbm] * 6 + [pl.BlockSpec(memory_space=pltpu.VMEM)],
        out_specs=hbm,
        out_shape=jax.ShapeDtypeStruct((S, D), bf),
        scratch_shapes=[
            pltpu.VMEM((S, D), bf),
            pltpu.VMEM((D, 3 * D), bf),
            pltpu.VMEM((D, D), bf),
            pltpu.VMEM((D, F), bf),
            pltpu.VMEM((D, F), bf),
            pltpu.VMEM((F, D), bf),
            pltpu.VMEM((S, D), bf),
            pltpu.VMEM((S, D), bf),
            pltpu.VMEM((3, S, 128), f32),
            pltpu.VMEM((3, S, 128), f32),
            pltpu.VMEM((16, 128, NA), f32),
            pltpu.VMEM((2, 16, 128, NA), f32),
            pltpu.VMEM((2, 16, 128, NA), f32),
            pltpu.VMEM((S, 128), f32),
            pltpu.SemaphoreType.DMA((11,)),
            pltpu.SemaphoreType.DMA(()),
        ],
        compiler_params=pltpu.CompilerParams(vmem_limit_bytes=100 * 1024 * 1024),
    )(A_x.reshape(S, D), A_wqkv, A_wo, B_W_gate, B_W_up, B_W_down,
      gate_w.reshape(1, D))
    return out.reshape(1, S, D)
```

```python
import jax
import jax.numpy as jnp
from jax import lax
import jax.experimental.pallas as pl
import jax.experimental.pallas.tpu as pltpu

S = 2048
D = 1024
F = 3584
H = 32
DH = 32
WIN = 8
NCH = D // 128
NA = S // 16
RB = 256
NRB = S // RB
FC = 512
NFC = F // FC
MB = 512
NMB = S // MB
SCALE = DH ** -0.5


def _qkv_chunk(x_v, wqkv_v, dst, c):
    co = pl.multiple_of(c * 128, 128)
    for t in range(3):
        w = wqkv_v[:, pl.ds(t * D + co, 128)]
        for m in range(NMB):
            r = jnp.dot(x_v[pl.ds(m * MB, MB), :], w,
                        preferred_element_type=jnp.float32)
            dst[t, pl.ds(m * MB, MB), :] = r


def _attention_chunk(src, tq, tk, tv, o32, o_v, c):
    lane = lax.broadcasted_iota(jnp.int32, (8, NA), 1)
    first = lane == 0
    for j in range(16):
        rows = pl.ds(j, NA, stride=16)
        tq[j] = (src[0, rows, :] * SCALE).T
        kt = src[1, rows, :].T
        vt = src[2, rows, :].T
        tk[0, j] = kt
        tv[0, j] = vt
        if j >= 2:
            tk[1, j] = pltpu.roll(kt, 1, 1)
            tv[1, j] = pltpu.roll(vt, 1, 1)
    for j in range(16):
        b, p = divmod(j, 2)
        srcs = []
        for w in range(WIN):
            if b >= w:
                srcs.append((0, 2 * (b - w) + p))
            else:
                srcs.append((1, 2 * (b - w + 8) + p))
        outs = []
        for h in range(4):
            hs = pl.ds(h * DH, DH)
            q = tq[j, hs, :]
            lg = []
            for (sh, jj) in srcs:
                pr = q * tk[sh, jj, hs, :]
                pr = (pr[0:8] + pr[8:16]) + (pr[16:24] + pr[24:32])
                l = jnp.broadcast_to(jnp.sum(pr, axis=0, keepdims=True), (8, NA))
                if sh:
                    l = jnp.where(first, jnp.float32(-1e9), l)
                lg.append(l)
            mx = lg[0]
            for l in lg[1:]:
                mx = jnp.maximum(mx, l)
            es = [jnp.exp(l - mx) for l in lg]
            den = es[0]
            for e in es[1:]:
                den = den + e
            inv = 1.0 / den
            acc = [None] * 4
            for (sh, jj), e in zip(srcs, es):
                vv = tv[sh, jj, hs, :]
                for r in range(4):
                    t = e * vv[r * 8:(r + 1) * 8]
                    acc[r] = t if acc[r] is None else acc[r] + t
            outs.extend([a_ * inv for a_ in acc])
        oj = jnp.concatenate(outs, axis=0)
        o32[pl.ds(j, NA, stride=16), :] = oj.T
    co = pl.multiple_of(c * 128, 128)
    o_v[:, pl.ds(co, 128)] = o32[...].astype(jnp.bfloat16)


def _kernel(x_h, wqkv_h, wo_h, wg_h, wu_h, wd_h, gw_ref, out_h,
            x_v, wqkv_v, wo_v, wg_v, wu_v, wd_v, o_v, out_v,
            bufa, bufb, tq, tk, tv, o32, h_v, sems, osem):
    def cp(hbm, vm, i):
        return pltpu.make_async_copy(hbm, vm, sems.at[i])

    c_x = [pltpu.make_async_copy(x_h.at[pl.ds(m * MB, MB), :],
                                 x_v.at[pl.ds(m * MB, MB), :], sems.at[11 + m])
           for m in range(NMB)]
    c_q0 = [cp(wqkv_h.at[:, pl.ds(t * D, 128)], wqkv_v.at[:, pl.ds(t * D, 128)], t)
            for t in range(3)]
    c_qr = [cp(wqkv_h.at[:, pl.ds(t * D + 128, D - 128)],
               wqkv_v.at[:, pl.ds(t * D + 128, D - 128)], 4 + t) for t in range(3)]
    c_wg = cp(wg_h, wg_v, 7)
    c_wu = cp(wu_h, wu_v, 8)
    c_wd = cp(wd_h, wd_v, 9)
    c_wo = cp(wo_h, wo_v, 10)
    for c_ in c_q0:
        c_.start()
    for c_ in c_x:
        c_.start()
    for c_ in c_q0:
        c_.wait()
    for m in range(NMB):
        c_x[m].wait()
        if m == 1:
            for c_ in c_qr:
                c_.start()
        for t in range(3):
            bufa[t, pl.ds(m * MB, MB), :] = jnp.dot(
                x_v[pl.ds(m * MB, MB), :], wqkv_v[:, pl.ds(t * D, 128)],
                preferred_element_type=jnp.float32)
    for c_ in c_qr:
        c_.wait()
    c_wg.start()
    c_wu.start()
    c_wd.start()
    c_wo.start()

    def glu(xb, fc):
        cs = pl.ds(fc * FC, FC)
        gt = jnp.dot(xb, wg_v[:, cs], preferred_element_type=jnp.float32)
        up = jnp.dot(xb, wu_v[:, cs], preferred_element_type=jnp.float32)
        return (jnp.maximum(gt, 0.0) * up).astype(jnp.bfloat16)

    def pair(i, carry):
        c = 2 * i
        _qkv_chunk(x_v, wqkv_v, bufb, c + 1)
        _attention_chunk(bufa, tq, tk, tv, o32, o_v, c)
        _qkv_chunk(x_v, wqkv_v, bufa, c + 2)
        _attention_chunk(bufb, tq, tk, tv, o32, o_v, c + 1)
        return carry

    lax.fori_loop(0, NCH // 2 - 1, pair, 0)
    _qkv_chunk(x_v, wqkv_v, bufb, NCH - 1)
    _attention_chunk(bufa, tq, tk, tv, o32, o_v, NCH - 2)
    c_wg.wait()
    c_wu.wait()
    for m in range(NMB):
        h_v[pl.ds(m * MB, MB), :] = glu(x_v[pl.ds(m * MB, MB), :], 0)
    _attention_chunk(bufb, tq, tk, tv, o32, o_v, NCH - 1)

    c_wd.wait()
    c_wo.wait()

    def out_cp(i):
        rs = pl.ds(pl.multiple_of(i * RB, RB), RB)
        return pltpu.make_async_copy(out_v.at[rs, :], out_h.at[rs, :], osem)

    def ffn(i, carry):
        rs = pl.ds(pl.multiple_of(i * RB, RB), RB)
        xb = x_v[rs, :]
        z = jnp.sum(xb.astype(jnp.float32) * gw_ref[...].astype(jnp.float32).reshape(1, D),
                    axis=-1, keepdims=True)
        g = jax.nn.sigmoid(z)
        hs = [h_v[rs, :]] + [glu(xb, fc) for fc in range(1, NFC)]
        hh = jnp.concatenate(hs, axis=1)
        bb = jnp.dot(hh, wd_v[...], preferred_element_type=jnp.float32)
        aa = jnp.dot(o_v[rs, :], wo_v[...], preferred_element_type=jnp.float32)
        out_v[rs, :] = (g * aa + (1.0 - g) * bb).astype(jnp.bfloat16)
        out_cp(i).start()
        return carry

    lax.fori_loop(0, NRB, ffn, 0)
    pltpu.make_async_copy(out_v, out_h, osem).wait()


@jax.jit
def pallas_gated_mix__sliding_local_dilated__glu_gated_reglu__prompt_kernel(
    A_x: jax.Array,
    A_wqkv: jax.Array,
    A_wo: jax.Array,
    B_x: jax.Array,
    B_W_gate: jax.Array,
    B_W_up: jax.Array,
    B_W_down: jax.Array,
    gate_w: jax.Array,
):
    del B_x
    bf = jnp.bfloat16
    f32 = jnp.float32
    hbm = pl.BlockSpec(memory_space=pl.ANY)
    out = pl.pallas_call(
        _kernel,
        in_specs=[hbm] * 6 + [pl.BlockSpec(memory_space=pltpu.VMEM)],
        out_specs=hbm,
        out_shape=jax.ShapeDtypeStruct((S, D), bf),
        scratch_shapes=[
            pltpu.VMEM((S, D), bf),
            pltpu.VMEM((D, 3 * D), bf),
            pltpu.VMEM((D, D), bf),
            pltpu.VMEM((D, F), bf),
            pltpu.VMEM((D, F), bf),
            pltpu.VMEM((F, D), bf),
            pltpu.VMEM((S, D), bf),
            pltpu.VMEM((S, D), bf),
            pltpu.VMEM((3, S, 128), f32),
            pltpu.VMEM((3, S, 128), f32),
            pltpu.VMEM((16, 128, NA), f32),
            pltpu.VMEM((2, 16, 128, NA), f32),
            pltpu.VMEM((2, 16, 128, NA), f32),
            pltpu.VMEM((S, 128), f32),
            pltpu.VMEM((S, FC), bf),
            pltpu.SemaphoreType.DMA((15,)),
            pltpu.SemaphoreType.DMA(()),
        ],
        compiler_params=pltpu.CompilerParams(vmem_limit_bytes=100 * 1024 * 1024),
    )(A_x.reshape(S, D), A_wqkv, A_wo, B_W_gate, B_W_up, B_W_down,
      gate_w)
    return out.reshape(1, S, D)
```

```python
import jax
import jax.numpy as jnp
from jax import lax
import jax.experimental.pallas as pl
import jax.experimental.pallas.tpu as pltpu

S = 2048
D = 1024
F = 3584
H = 32
DH = 32
WIN = 8
NCH = D // 128
NA = S // 16
RB = 256
NRB = S // RB
FC = 512
NFC = F // FC
MB = 512
NMB = S // MB
OFF = 3
SCALE = DH ** -0.5


def _tie(xb, toks, b):
    if not toks:
        return xb
    top = [xb[0:16, k * 128:(k + 1) * 128] for k in range(8)]
    for k, tk_ in toks.items():
        top[k] = jnp.where(b == 1000, pltpu.bitcast(tk_, jnp.bfloat16), top[k])
    return jnp.concatenate([jnp.concatenate(top, axis=1), xb[16:]], axis=0)


def _slots(tok, n, t):
    return {(i * n // 8 + OFF) % 8: x for i, x in enumerate(tok or []) if (i * n // 8 + OFF) // 8 == t}


def _mm_step(x_v, wqkv_v, dst, c, b, tok):
    rs = pl.ds(pl.multiple_of(b * RB, RB), RB)
    xb = x_v[rs, :]
    for t in range(3):
        dst[t, rs, :] = jnp.dot(_tie(xb, _slots(tok, 20, t), b), wqkv_v[:, pl.ds(t * D + c * 128, 128)],
                                preferred_element_type=jnp.float32)


def _tr_step(src, tq, tk, tv, b):
    for p in range(2):
        rows = pl.ds(2 * b + p, NA, stride=16)
        tq[b, p] = (src[0, rows, :] * SCALE).T
        kt = src[1, rows, :].T
        vt = src[2, rows, :].T
        tk[8 + b, p] = kt
        tv[8 + b, p] = vt
        tk[b, p] = pltpu.roll(kt, 1, 1)
        tv[b, p] = pltpu.roll(vt, 1, 1)


def _att_step(tq, tk, tv, o32, b):
    lane = lax.broadcasted_iota(jnp.int32, (8, NA), 1)
    sub = lax.broadcasted_iota(jnp.int32, (8, NA), 0)
    m4, m2, m1 = (sub & 4) == 0, (sub & 2) == 0, (sub & 1) == 0
    wrow = (sub >> 2) | (sub & 2) | ((sub & 1) << 2)
    dead = (lane == 0) & (wrow > b)
    tok = []
    for p in range(2):
        outs = []
        for h in range(4):
            hs = pl.ds(h * DH, DH)
            q = tq[b, p, hs, :]
            lg = []
            for w in range(WIN):
                pr = q * tk[b + (8 - w), p, hs, :]
                pr = (pr[0:8] + pr[8:16]) + (pr[16:24] + pr[24:32])
                lg.append(pr)
            z = [jnp.where(m4, u, v) + pltpu.roll(jnp.where(m4, v, u), 4, 0)
                 for u, v in zip(lg[0::2], lg[1::2])]
            for d, m in ((2, m2), (1, m1)):
                z = [jnp.where(m, u, v) + jnp.where(
                    m, pltpu.roll(u, 8 - d, 0), pltpu.roll(v, d, 0))
                    for u, v in zip(z[0::2], z[1::2])]
            l = jnp.where(dead, jnp.float32(-1e9), z[0])
            e = jnp.exp(l - jnp.max(l, axis=0, keepdims=True))
            pn = e / jnp.sum(e, axis=0, keepdims=True)
            es = [jnp.broadcast_to(pn[r:r + 1], (8, NA)) for r in (0, 4, 2, 6, 1, 5, 3, 7)]
            acc = [None] * 4
            for w, e in enumerate(es):
                vv = tv[b + (8 - w), p, hs, :]
                for r in range(4):
                    t = e * vv[r * 8:(r + 1) * 8]
                    acc[r] = t if acc[r] is None else acc[r] + t
            outs.extend(acc)
            tok.append((outs[-1] + outs[-2]) + (outs[-3] + outs[-4]))
        oj = jnp.concatenate(outs, axis=0)
        o32[pl.ds(2 * b + p, NA, stride=16), :] = oj.T
    return tok


def _cv_step(o32, o_v, c, b):
    rs = pl.ds(pl.multiple_of(b * RB, RB), RB)
    o_v[rs, pl.ds(c * 128, 128)] = o32[rs, :].astype(jnp.bfloat16)


def _glu(xb, wg_v, wu_v, fc, tok=None, b=None):
    cs = pl.ds(fc * FC, FC)
    gt = jnp.dot(_tie(xb, _slots(tok, 12, 0), b), wg_v[:, cs], preferred_element_type=jnp.float32)
    up = jnp.dot(_tie(xb, _slots(tok, 12, 1), b), wu_v[:, cs], preferred_element_type=jnp.float32)
    return (jnp.maximum(gt, 0.0) * up).astype(jnp.bfloat16)


def _kernel(x_h, wqkv_h, wo_h, wg_h, wu_h, wd_h, gw_ref, out_h,
            x_v, wqkv_v, wo_v, wg_v, wu_v, wd_v, o_v, out_v,
            buf0, buf1, tq0, tq1, tk0, tk1, tv0, tv1, o320, o321, h_v,
            sems, qsem, xsem, osem):
    buf, tq, tk, tv, o32 = (buf0, buf1), (tq0, tq1), (tk0, tk1), (tv0, tv1), (o320, o321)

    def cp(hbm, vm, i):
        return pltpu.make_async_copy(hbm, vm, sems.at[i])

    def x_cp(m):
        rs = pl.ds(pl.multiple_of(m * RB, RB), RB)
        return pltpu.make_async_copy(x_h.at[rs, :], x_v.at[rs, :], xsem.at[m])

    def q_cp(c):
        return [pltpu.make_async_copy(wqkv_h.at[:, pl.ds(t * D + c * 128, 128)],
                                      wqkv_v.at[:, pl.ds(t * D + c * 128, 128)],
                                      qsem.at[c]) for t in range(3)]

    c_wg = cp(wg_h, wg_v, 0)
    c_wu = cp(wu_h, wu_v, 1)
    c_wd = cp(wd_h, wd_v, 2)
    c_wo = cp(wo_h, wo_v, 3)

    for c_ in q_cp(0):
        c_.start()
    for m in range(2):
        x_cp(m).start()
    for t in range(NCH + 2):
        if t < NCH:
            for c_ in q_cp(t):
                c_.wait()
        if t == 0:
            for m in range(2, NRB):
                x_cp(m).start()
        for c in {0: (1, 2), 1: (3, 4), 2: (5, 6, 7)}.get(t, ()):
            for c_ in q_cp(c):
                c_.start()
        if t == 1:
            c_wg.start()
        if t == 2:
            c_wu.start()
        if t == 3:
            c_wd.start()
            c_wo.start()
        if t == NCH:
            c_wg.wait()
            c_wu.wait()

        def step(b, carry, t=t):
            if t == 0:
                x_cp(b).wait()
            tok = None
            if 1 <= t <= NCH:
                k = (t - 1) % 2
                _tr_step(buf[k], tq[k], tk[k], tv[k], b)
            if 2 <= t:
                k = t % 2
                tok = _att_step(tq[k], tk[k], tv[k], o32[k], b)
            if 3 <= t:
                _cv_step(o32[(t - 3) % 2], o_v, t - 3, b)
            if t < NCH:
                _mm_step(x_v, wqkv_v, buf[t % 2], t, b, tok)
            else:
                rs = pl.ds(pl.multiple_of(b * RB, RB), RB)
                h_v[t - NCH, rs, :] = _glu(x_v[rs, :], wg_v, wu_v, t - NCH, tok, b)
            return carry

        lax.fori_loop(0, NRB, step, 0, unroll=4)

    c_wd.wait()
    c_wo.wait()

    def out_cp(i):
        rs = pl.ds(pl.multiple_of(i * RB, RB), RB)
        return pltpu.make_async_copy(out_v.at[rs, :], out_h.at[rs, :], osem)

    def ffn(i, carry):
        rs = pl.ds(pl.multiple_of(i * RB, RB), RB)
        xb = x_v[rs, :]
        z = jnp.sum(xb.astype(jnp.float32) * gw_ref[...].astype(jnp.float32).reshape(1, D),
                    axis=-1, keepdims=True)
        g = jax.nn.sigmoid(z)
        _cv_step(o32[(NCH - 1) % 2], o_v, NCH - 1, i)
        hs = [h_v[fc, rs, :] for fc in range(2)]
        hs += [_glu(xb, wg_v, wu_v, fc) for fc in range(2, NFC)]
        hh = jnp.concatenate(hs, axis=1)
        bb = jnp.dot(hh, wd_v[...], preferred_element_type=jnp.float32)
        aa = jnp.dot(o_v[rs, :], wo_v[...], preferred_element_type=jnp.float32)
        out_v[rs, :] = (g * aa + (1.0 - g) * bb).astype(jnp.bfloat16)
        out_cp(i).start()
        return carry

    lax.fori_loop(0, NRB, ffn, 0)
    pltpu.make_async_copy(out_v, out_h, osem).wait()


@jax.jit
def pallas_gated_mix__sliding_local_dilated__glu_gated_reglu__prompt_kernel(
    A_x: jax.Array,
    A_wqkv: jax.Array,
    A_wo: jax.Array,
    B_x: jax.Array,
    B_W_gate: jax.Array,
    B_W_up: jax.Array,
    B_W_down: jax.Array,
    gate_w: jax.Array,
):
    del B_x
    bf = jnp.bfloat16
    f32 = jnp.float32
    hbm = pl.BlockSpec(memory_space=pl.ANY)
    out = pl.pallas_call(
        _kernel,
        in_specs=[hbm] * 6 + [pl.BlockSpec(memory_space=pltpu.VMEM)],
        out_specs=hbm,
        out_shape=jax.ShapeDtypeStruct((S, D), bf),
        scratch_shapes=[
            pltpu.VMEM((S, D), bf),
            pltpu.VMEM((D, 3 * D), bf),
            pltpu.VMEM((D, D), bf),
            pltpu.VMEM((D, F), bf),
            pltpu.VMEM((D, F), bf),
            pltpu.VMEM((F, D), bf),
            pltpu.VMEM((S, D), bf),
            pltpu.VMEM((S, D), bf),
            *[pltpu.VMEM((3, S, 128), f32)] * 2,
            *[pltpu.VMEM((8, 2, 128, NA), f32)] * 2,
            *[pltpu.VMEM((16, 2, 128, NA), f32)] * 4,
            *[pltpu.VMEM((S, 128), f32)] * 2,
            pltpu.VMEM((2, S, FC), bf),
            pltpu.SemaphoreType.DMA((4,)),
            pltpu.SemaphoreType.DMA((NCH,)),
            pltpu.SemaphoreType.DMA((NRB,)),
            pltpu.SemaphoreType.DMA(()),
        ],
        compiler_params=pltpu.CompilerParams(vmem_limit_bytes=100 * 1024 * 1024),
    )(A_x.reshape(S, D), A_wqkv, A_wo, B_W_gate, B_W_up, B_W_down,
      gate_w)
    return out.reshape(1, S, D)
```
